```python
import os as _os
_os.environ.setdefault("JAX_PLATFORMS", "cpu")
import jax
import jax.numpy as jnp

def _softmax(x, axis=-1):
    return jax.nn.softmax(x, axis=axis)
def _gelu(x):
    return jax.nn.gelu(x, approximate=True)
def _silu(x):
    return jax.nn.silu(x)
def _sigmoid(x):
    return jax.nn.sigmoid(x)
def _layernorm(x, axis=-1, eps=1e-5):
    m = jnp.mean(x, axis=axis, keepdims=True)
    v = jnp.var(x, axis=axis, keepdims=True)
    return (x - m) / jnp.sqrt(v + eps)
def _scatter_add(tgt, idx, src, axis=0):
    return tgt.at[idx].add(src)
def _segment_sum(src, seg, n):
    return jax.ops.segment_sum(src, seg, n)
class _Rng:
    def __init__(self, key):
        self._k = key
    def _next(self):
        self._k, sub = jax.random.split(self._k)
        return sub
    def normal(self, shape):
        return jax.random.normal(self._next(), shape, dtype=jnp.bfloat16)
    def randint(self, lo, hi, shape):
        return jax.random.randint(self._next(), shape, lo, hi, dtype=jnp.int32)
    def uniform(self, shape, lo=0.0, hi=1.0):
        return jax.random.uniform(self._next(), shape, jnp.bfloat16, lo, hi)
    def permutation(self, n):
        return jax.random.permutation(self._next(), n)


kernel_name = 'concat_heads__sliding_block_cached__compressed_kv_cla__decode'

def setup_inputs():
    _rng = _Rng(jax.random.key(int.from_bytes(__import__("os").urandom(4), "little")))
    _w = (lambda a: (lambda t: t.astype(jnp.bfloat16) if jnp.issubdtype(t.dtype, jnp.floating) else t)(jnp.asarray(a)))
    def _A_setup():
        B, Sq, D = 1, 1, 512
        Hq, Hkv, Sk, Dh = 32, 32, 4096, 128
        assert Hq % Hkv == 0, (Hq, Hkv)
        return {
            "x": _w((lambda *s: _rng.normal(s) * 0.8)(B, Sq, D)),
            "k_cache": _w((lambda *s: _rng.normal(s) * 0.8)(B, Hkv, Sk, Dh)),
            "v_cache": _w((lambda *s: _rng.normal(s) * 0.05)(B, Hkv, Sk, Dh)),
            "wq": _w((lambda *s: _rng.normal(s) * 0.8)(D, Hq * Dh) * (D ** -0.5)),
            "wo": _w((lambda *s: _rng.normal(s) * 0.05)(Hq * Dh, D) * ((Hq * Dh) ** -0.5)),
        }
    _A_in = _A_setup()

    def _B_setup():
        B, H, Sq, Sk, D, M = 1, 32, 1, 4096, 128, 512
        Dc = 4 * D
        return {
            "x": _w((lambda *s: _rng.normal(s) * 1.6)(B, Sq, M)),
            "c_kv": _w((lambda *s: _rng.normal(s) * 0.1)(B, Sk, Dc)),
            "w_q": _w((lambda *s: _rng.normal(s) * 1.6)(M, H, D) * (M ** -0.5)),
            "w_uk": _w((lambda *s: _rng.normal(s) * 1.6)(Dc, H, D) * (Dc ** -0.5)),
            "w_uv": _w((lambda *s: _rng.normal(s) * 0.1)(Dc, H, D) * (Dc ** -0.5)),
            "w_o": _w((lambda *s: _rng.normal(s) * 0.1)(H, D, M) * ((H * D) ** -0.5)),
        }
    _B_in = _B_setup()

    return {
        "A_x": _A_in["x"],
        "A_k_cache": _A_in["k_cache"],
        "A_v_cache": _A_in["v_cache"],
        "A_wq": _A_in["wq"],
        "A_wo": _A_in["wo"],
        "B_x": _B_in["x"],
        "B_c_kv": _B_in["c_kv"],
        "B_w_q": _B_in["w_q"],
        "B_w_uk": _B_in["w_uk"],
        "B_w_uv": _B_in["w_uv"],
        "B_w_o": _B_in["w_o"],
    }

def reference(A_x, A_k_cache, A_v_cache, A_wq, A_wo, B_x, B_c_kv, B_w_q, B_w_uk, B_w_uv, B_w_o):
    def _A_ref(x, k_cache, v_cache, wq, wo):
        B, Sq, D = x.shape
        Hq, Dh = 32, 128
        Hkv, Sk = k_cache.shape[1], k_cache.shape[2]
        W = min(4096, max(256, Sk // 4))
        rep = Hq // Hkv
        q = (lambda x, *d: x.transpose(*d))((x @ wq).reshape(B, Sq, Hq, Dh), 0, 2, 1, 3)
        k = jnp.repeat(k_cache[:, :, Sk - W:, :], rep, axis=1)
        v = jnp.repeat(v_cache[:, :, Sk - W:, :], rep, axis=1)
        scores = jnp.einsum("bhqd,bhkd->bhqk", q, k) * (Dh ** -0.5)
        p = _softmax(scores, axis=-1)
        o = jnp.einsum("bhqk,bhkd->bhqd", p, v)
        return (lambda x, *d: x.transpose(*d))(o, 0, 2, 1, 3).reshape(B, Sq, Hq * Dh) @ wo

    def _B_ref(x, c_kv, w_q, w_uk, w_uv, w_o):
        B, Sq, M = x.shape[0], x.shape[1], x.shape[2]
        Sk = c_kv.shape[1]
        H, D = w_q.shape[1], w_q.shape[2]
        q = jnp.einsum("bqm,mhd->bhqd", x, w_q)
        k = jnp.einsum("bkc,chd->bhkd", c_kv, w_uk)
        v = jnp.einsum("bkc,chd->bhkd", c_kv, w_uv)
        scores = jnp.einsum("bhqd,bhkd->bhqk", q, k) * (D ** -0.5)
        off = Sk - Sq
        qi = jnp.arange(Sq)[:, None]
        kj = jnp.arange(Sk)[None, :]
        cmask = kj <= (qi + off)
        scores = jnp.where(cmask[None, None], scores, -1e9)
        p = _softmax(scores, axis=-1)
        ctx = jnp.einsum("bhqk,bhkd->bhqd", p, v)
        return jnp.einsum("bhqd,hdm->bqm", ctx, w_o)

    a = _A_ref(A_x, A_k_cache, A_v_cache, A_wq, A_wo)
    b = _B_ref(B_x, B_c_kv, B_w_q, B_w_uk, B_w_uv, B_w_o)
    return jnp.concatenate([a, b], axis=-1)
```

```python
import jax
import jax.numpy as jnp
from jax import lax
import jax.experimental.pallas as pl
import jax.experimental.pallas.tpu as pltpu

H = 32
D = 128
M = 512
SK = 4096
W = 1024
C = 512
F32 = jnp.float32
BF16 = jnp.bfloat16
NT = (((1,), (1,)), ((), ()))

WO_SPLITS = (3456, 512, 128)


def _kernel(ax_hbm, ak_hbm, av_hbm, awq_hbm, awo_hbm, bx_hbm, bc_hbm, bwq_hbm, bwuk_hbm, bwuv_hbm, bwo_hbm,
            out_ref,
            ax_v, bx_v, k_v, v_v, awq_v, awo_v, c_v, bwq_v, bwuk_v, bwuv_v, bwo_v, sems):
    scale = D ** -0.5
    cps = {}
    def mk(name, src, dst):
        cps[name] = pltpu.make_async_copy(src, dst, sems.at[len(cps)])
    mk('bwq', bwq_hbm, bwq_v)
    mk('bx', bx_hbm, bx_v)
    mk('ax', ax_hbm, ax_v)
    mk('bwuk', bwuk_hbm, bwuk_v)
    mk('c', bc_hbm, c_v)
    mk('awq', awq_hbm, awq_v)
    mk('k', ak_hbm.at[0, :, pl.ds(SK - W, W), :], k_v)
    mk('v', av_hbm.at[0, :, pl.ds(SK - W, W), :], v_v)
    mk('bwuv', bwuv_hbm, bwuv_v)
    mk('bwo', bwo_hbm, bwo_v)
    r0 = 0
    for i, r in enumerate(WO_SPLITS):
        mk('awo%d' % i, awo_hbm.at[pl.ds(r0, r), :], awo_v.at[pl.ds(r0, r), :])
        r0 += r
    for c in cps.values():
        c.start()

    et = (lax.broadcasted_iota(jnp.int32, (128, 4096), 1) // 32 ==
          lax.broadcasted_iota(jnp.int32, (128, 4096), 0)).astype(BF16)
    dmask = (lax.broadcasted_iota(jnp.int32, (32, 4096), 1) % 32 ==
             lax.broadcasted_iota(jnp.int32, (32, 4096), 0))

    def expand_matmul(y, w_ref):
        ys = jnp.concatenate([y[:, t * 128:(t + 1) * 128] for t in range(4)], axis=0)
        ye = jnp.dot(ys, et, preferred_element_type=F32)
        return [jnp.where(dmask, ye[t * 32:(t + 1) * 32, :], 0.0).astype(BF16) for t in range(4)]

    cps['bx'].wait()
    xb = jnp.broadcast_to(bx_v[0], (32, M))
    xq = expand_matmul(xb, None)
    cps['bwq'].wait()
    qb = jnp.zeros((32, 128), F32)
    for t in range(4):
        qb = qb + jnp.dot(xq[t], bwq_v[pl.ds(t * 4096, 4096), :], preferred_element_type=F32)
    qb = qb.astype(BF16)

    cps['bwuk'].wait()
    rm = []
    for t in range(4):
        r = lax.dot_general(qb, bwuk_v[pl.ds(t * 4096, 4096), :], NT, preferred_element_type=F32)
        rm.append(jnp.where(dmask, r, 0.0).astype(BF16))
    rs = jnp.concatenate(rm, axis=0)
    qa_s = lax.dot_general(rs, et, NT, preferred_element_type=F32)
    qabs = jnp.concatenate([qa_s[t * 32:(t + 1) * 32, :] for t in range(4)], axis=1).astype(BF16)

    cps['c'].wait()
    sb = lax.dot_general(qabs, c_v[...], NT, preferred_element_type=F32) * scale
    mb = jnp.max(sb, axis=1, keepdims=True)
    eb = jnp.exp(sb - mb)
    lb = jnp.sum(eb, axis=1, keepdims=True)
    cc = jnp.dot(eb.astype(BF16), c_v[...], preferred_element_type=F32) / lb
    xv = expand_matmul(cc.astype(BF16), None)

    cps['ax'].wait()
    cps['awq'].wait()
    xa = jnp.broadcast_to(ax_v[0], (8, M))
    qa = jnp.dot(xa, awq_v[...], preferred_element_type=F32)
    row8 = lax.broadcasted_iota(jnp.int32, (8, 4096), 0)
    hm = (lax.broadcasted_iota(jnp.int32, (8, 4096), 1) // 128) % 8 == row8
    qm = jnp.where(hm, qa, 0.0).astype(BF16)

    cps['k'].wait()
    ps = []
    for g in range(4):
        s = jnp.zeros((8, W), F32)
        for j in range(8):
            h = g * 8 + j
            s = s + lax.dot_general(qm[:, h * 128:(h + 1) * 128], k_v[h], NT, preferred_element_type=F32)
        s = s * scale
        m = jnp.max(s, axis=1, keepdims=True)
        e = jnp.exp(s - m)
        l = jnp.sum(e, axis=1, keepdims=True)
        ps.append((e.astype(BF16), l))

    cps['v'].wait()
    r8 = lax.broadcasted_iota(jnp.int32, (8, 128), 0)
    oms = []
    for g in range(4):
        e, l = ps[g]
        inv = 1.0 / l
        for j in range(8):
            h = g * 8 + j
            o = jnp.dot(e, v_v[h], preferred_element_type=F32) * inv
            oms.append(jnp.where(r8 == j, o, 0.0))
    om = jnp.concatenate(oms, axis=1)
    oa = jnp.sum(om, axis=0, keepdims=True).astype(BF16)
    oa = jnp.broadcast_to(oa, (8, 4096))

    cps['bwuv'].wait()
    cx = jnp.zeros((32, 128), F32)
    for t in range(4):
        cx = cx + jnp.dot(xv[t], bwuv_v[pl.ds(t * 4096, 4096), :], preferred_element_type=F32)
    cxm = jnp.concatenate([jnp.where(r8 == (h % 8), cx[(h // 8) * 8:(h // 8) * 8 + 8, :], 0.0) for h in range(32)], axis=1).astype(BF16)

    cps['bwo'].wait()
    ob = jnp.sum(jnp.dot(cxm, bwo_v[...], preferred_element_type=F32), axis=0, keepdims=True)
    out_ref[0, :, M:] = ob.astype(out_ref.dtype)

    acc = jnp.zeros((8, M), F32)
    r0 = 0
    for i, r in enumerate(WO_SPLITS):
        cps['awo%d' % i].wait()
        acc = acc + jnp.dot(oa[:, r0:r0 + r], awo_v[pl.ds(r0, r), :], preferred_element_type=F32)
        r0 += r
    out_ref[0, :, :M] = acc[0:1, :].astype(out_ref.dtype)


@jax.jit
def pallas_concat_heads__sliding_block_cached__compressed_kv_cla__decode_kernel(A_x, A_k_cache, A_v_cache, A_wq, A_wo, B_x, B_c_kv, B_w_q, B_w_uk, B_w_uv, B_w_o):
    ncp = 10 + len(WO_SPLITS)
    return pl.pallas_call(
        _kernel,
        out_shape=jax.ShapeDtypeStruct((1, 1, 2 * M), BF16),
        in_specs=[pl.BlockSpec(memory_space=pl.ANY)] * 11,
        out_specs=pl.BlockSpec(memory_space=pltpu.VMEM),
        scratch_shapes=[
            pltpu.VMEM((1, 1, M), BF16),
            pltpu.VMEM((1, 1, M), BF16),
            pltpu.VMEM((H, W, D), BF16),
            pltpu.VMEM((H, W, D), BF16),
            pltpu.VMEM((M, H * D), BF16),
            pltpu.VMEM((H * D, M), BF16),
            pltpu.VMEM((SK, C), BF16),
            pltpu.VMEM((M * H, D), BF16),
            pltpu.VMEM((C * H, D), BF16),
            pltpu.VMEM((C * H, D), BF16),
            pltpu.VMEM((H * D, M), BF16),
            pltpu.SemaphoreType.DMA((ncp,)),
        ],
        compiler_params=pltpu.CompilerParams(vmem_limit_bytes=100 * 1024 * 1024),
    )(A_x, A_k_cache, A_v_cache, A_wq, A_wo, B_x,
      B_c_kv.reshape(SK, C), B_w_q.reshape(M * H, D), B_w_uk.reshape(C * H, D),
      B_w_uv.reshape(C * H, D), B_w_o.reshape(H * D, M))
```

```python
import jax
import jax.numpy as jnp
from jax import lax
import jax.experimental.pallas as pl
import jax.experimental.pallas.tpu as pltpu

H = 32
D = 128
M = 512
SK = 4096
W = 1024
C = 512
HD = H * D
F32 = jnp.float32
BF16 = jnp.bfloat16
NT = (((1,), (1,)), ((), ()))

WO_GROUPS = (
    ((112,) * 9, 1040),
    ((112,), 1296),
    ((), 384),
    ((), 128),
)
WO_VPU = (96, 32)
NSLOT = 3
UNITS = tuple(u for g, _ in WO_GROUPS for u in g)
N_MAIN = 12 + len(WO_GROUPS) + len(WO_VPU)
assert sum(UNITS) + sum(r for _, r in WO_GROUPS) + sum(WO_VPU) == HD
assert sum(WO_VPU) <= D and all((sum(g) + r) % 128 == 0 for g, r in WO_GROUPS)


def _body(ax_hbm, ak_hbm, av_hbm, awq_hbm, awo_hbm, bx_hbm, bc_hbm, bwq_hbm, bwuk_hbm,
          bwuv_hbm, bwo_hbm, out_ref,
          ax_v, bx_v, k_v, v_v, awq_v, awo_v, c_v, bwq_v, bwuk_v, bwuv_v, bwo_v,
          acc_v, ocol_v, sm, sems, bsems):
    scale = D ** -0.5
    hh = H // 2

    main = {}

    def mk(name, src, dst):
        main[name] = pltpu.make_async_copy(src, dst, sems.at[len(main)])

    mk('bwq', bwq_hbm, bwq_v)
    mk('bx', bx_hbm, bx_v)
    mk('ax', ax_hbm, ax_v)
    mk('bwuk', bwuk_hbm, bwuk_v)
    mk('c', bc_hbm, c_v)
    mk('awq', awq_hbm, awq_v)
    for name, src, dst in (('k', ak_hbm, k_v), ('v', av_hbm, v_v)):
        for i in range(2):
            mk(name + str(i), src.at[0, pl.ds(i * hh, hh), pl.ds(SK - W, W), :],
               dst.at[pl.ds(i * hh, hh)])
    mk('bwuv', bwuv_hbm, bwuv_v)
    mk('bwo', bwo_hbm, bwo_v)

    nu = len(UNITS)
    h2s, s2v = [], []
    r0 = 0
    for g, (units, direct) in enumerate(WO_GROUPS):
        for r in units:
            i = len(h2s)
            slot = sm.at[i % NSLOT, pl.ds(0, r), :]
            h2s.append(pltpu.make_async_copy(awo_hbm.at[pl.ds(r0, r), :], slot, bsems.at[i]))
            s2v.append(pltpu.make_async_copy(slot, awo_v.at[pl.ds(r0, r), :], bsems.at[nu + i]))
            r0 += r
        mk('wo%d' % g, awo_hbm.at[pl.ds(r0, direct), :], awo_v.at[pl.ds(r0, direct), :])
        r0 += direct
    for i, r in enumerate(WO_VPU):
        mk('wov%d' % i, awo_hbm.at[pl.ds(r0, r), :], awo_v.at[pl.ds(r0, r), :])
        r0 += r
    assert len(main) == N_MAIN

    n_sync = [0]
    s2v_done = set()

    def wait_s2v(i):
        if i not in s2v_done:
            s2v[i].wait()
            s2v_done.add(i)

    def sync():
        i = n_sync[0]
        n_sync[0] = i + 1
        if 1 <= i <= nu:
            h2s[i - 1].wait()
            s2v[i - 1].start()
        if i < nu:
            if i >= NSLOT:
                wait_s2v(i - NSLOT)
            h2s[i].start()

    def arrive(name):
        main[name].wait()
        sync()

    for cp in main.values():
        cp.start()
    sync()

    et = (lax.broadcasted_iota(jnp.int32, (128, 128 * H), 1) // H ==
          lax.broadcasted_iota(jnp.int32, (128, 128 * H), 0)).astype(BF16)
    dmask = (lax.broadcasted_iota(jnp.int32, (H, 128 * H), 1) % H ==
             lax.broadcasted_iota(jnp.int32, (H, 128 * H), 0))
    row8 = lax.broadcasted_iota(jnp.int32, (8, D), 0)

    def expand(y):
        ys = jnp.concatenate([y[:, t * 128:(t + 1) * 128] for t in range(4)], axis=0)
        ye = jnp.dot(ys, et, preferred_element_type=F32)
        return [jnp.where(dmask, ye[t * H:(t + 1) * H, :], 0.0).astype(BF16) for t in range(4)]

    def head_matmul(blocks, w_ref):
        acc = jnp.zeros((H, D), F32)
        for t in range(4):
            acc = acc + jnp.dot(blocks[t], w_ref[pl.ds(t * 128 * H, 128 * H), :],
                                preferred_element_type=F32)
        return acc

    arrive('bwq')
    main['bx'].wait()
    qb = head_matmul(expand(jnp.broadcast_to(bx_v[0], (H, M))), bwq_v).astype(BF16)

    arrive('bwuk')
    rm = []
    for t in range(4):
        r = lax.dot_general(qb, bwuk_v[pl.ds(t * 128 * H, 128 * H), :], NT,
                            preferred_element_type=F32)
        rm.append(jnp.where(dmask, r, 0.0).astype(BF16))
    qa_s = lax.dot_general(jnp.concatenate(rm, axis=0), et, NT, preferred_element_type=F32)
    qabs = jnp.concatenate([qa_s[t * H:(t + 1) * H, :] for t in range(4)], axis=1).astype(BF16)

    arrive('c')
    sb = lax.dot_general(qabs, c_v[...], NT, preferred_element_type=F32) * scale
    eb = jnp.exp(sb - jnp.max(sb, axis=1, keepdims=True))
    lb = jnp.sum(eb, axis=1, keepdims=True)
    cc = jnp.dot(eb.astype(BF16), c_v[...], preferred_element_type=F32) / lb
    xv = expand(cc.astype(BF16))

    arrive('awq')
    main['ax'].wait()
    qa = jnp.dot(jnp.broadcast_to(ax_v[0], (8, M)), awq_v[...], preferred_element_type=F32)
    hmask = ((lax.broadcasted_iota(jnp.int32, (8, HD), 1) // D) % 8 ==
             lax.broadcasted_iota(jnp.int32, (8, HD), 0))
    qm = jnp.where(hmask, qa, 0.0).astype(BF16)

    arrive('k0')
    arrive('k1')
    ps = []
    for g in range(H // 8):
        s = jnp.zeros((8, W), F32)
        for h in range(8 * g, 8 * g + 8):
            s = s + lax.dot_general(qm[:, h * D:(h + 1) * D], k_v[h], NT,
                                    preferred_element_type=F32)
        s = s * scale
        e = jnp.exp(s - jnp.max(s, axis=1, keepdims=True))
        ps.append((e.astype(BF16), 1.0 / jnp.sum(e, axis=1, keepdims=True)))

    arrive('v0')
    arrive('v1')
    oms = []
    for h in range(H):
        e, inv = ps[h // 8]
        o = jnp.dot(e, v_v[h], preferred_element_type=F32) * inv
        oms.append(jnp.where(row8 == h % 8, o, 0.0).astype(BF16))
    om = jnp.concatenate(oms, axis=1)
    olast = oms[H - 1].astype(F32)[7:8, :]
    ocol_v[...] = jnp.broadcast_to(olast, (D, D)).T

    arrive('bwuv')
    cx = head_matmul(xv, bwuv_v)
    cxm = jnp.concatenate(
        [jnp.where(row8 == h % 8, cx[(h // 8) * 8:(h // 8) * 8 + 8, :], 0.0) for h in range(H)],
        axis=1).astype(BF16)
    arrive('bwo')
    ob = jnp.sum(jnp.dot(cxm, bwo_v[...], preferred_element_type=F32), axis=0, keepdims=True)
    out_ref[0, :, M:] = ob.astype(out_ref.dtype)

    assert n_sync[0] > nu
    r0 = 0
    u0 = 0
    for g, (units, direct) in enumerate(WO_GROUPS):
        main['wo%d' % g].wait()
        for i in range(u0, u0 + len(units)):
            wait_s2v(i)
        u0 += len(units)
        r = sum(units) + direct
        part = jnp.dot(om[:, r0:r0 + r], awo_v[pl.ds(r0, r), :], preferred_element_type=F32)
        acc_v[...] = part if g == 0 else part + acc_v[...]
        r0 += r
    for i, r in enumerate(WO_VPU):
        main['wov%d' % i].wait()
        part = acc_v[...]
        for rr in range(r0, r0 + r, 8):
            oc = ocol_v[pl.ds(rr - (HD - D), 8), :]
            part = part + (awo_v[pl.ds(rr, 8), :].astype(F32) *
                           jnp.concatenate([oc] * (M // D), axis=1))
        if i + 1 < len(WO_VPU):
            acc_v[...] = part
        else:
            out_ref[0, :, :M] = jnp.sum(part, axis=0, keepdims=True).astype(out_ref.dtype)
        r0 += r


def _kernel(*refs):
    pl.run_scoped(lambda sems, bsems: _body(*refs, sems, bsems),
                  pltpu.SemaphoreType.DMA((N_MAIN,)),
                  pltpu.SemaphoreType.DMA((2 * len(UNITS),)))


@jax.jit
def pallas_concat_heads__sliding_block_cached__compressed_kv_cla__decode_kernel(
    A_x: jax.Array,
    A_k_cache: jax.Array,
    A_v_cache: jax.Array,
    A_wq: jax.Array,
    A_wo: jax.Array,
    B_x: jax.Array,
    B_c_kv: jax.Array,
    B_w_q: jax.Array,
    B_w_uk: jax.Array,
    B_w_uv: jax.Array,
    B_w_o: jax.Array,
):
    return pl.pallas_call(
        _kernel,
        out_shape=jax.ShapeDtypeStruct((1, 1, 2 * M), BF16),
        in_specs=[pl.BlockSpec(memory_space=pl.ANY)] * 11,
        out_specs=pl.BlockSpec(memory_space=pltpu.VMEM),
        scratch_shapes=[
            pltpu.VMEM((1, 1, M), BF16),
            pltpu.VMEM((1, 1, M), BF16),
            pltpu.VMEM((H, W, D), BF16),
            pltpu.VMEM((H, W, D), BF16),
            pltpu.VMEM((M, HD), BF16),
            pltpu.VMEM((HD, M), BF16),
            pltpu.VMEM((SK, C), BF16),
            pltpu.VMEM((M * H, D), BF16),
            pltpu.VMEM((C * H, D), BF16),
            pltpu.VMEM((C * H, D), BF16),
            pltpu.VMEM((HD, M), BF16),
            pltpu.VMEM((8, M), F32),
            pltpu.VMEM((D, D), F32),
            pltpu.SMEM((NSLOT, max(UNITS), M), BF16),
        ],
        compiler_params=pltpu.CompilerParams(vmem_limit_bytes=100 * 1024 * 1024),
    )(A_x, A_k_cache, A_v_cache, A_wq, A_wo, B_x,
      B_c_kv.reshape(SK, C), B_w_q.reshape(M * H, D), B_w_uk.reshape(C * H, D),
      B_w_uv.reshape(C * H, D), B_w_o.reshape(HD, M))
```

```python
import jax
import jax.numpy as jnp
from jax import lax
import jax.experimental.pallas as pl
import jax.experimental.pallas.tpu as pltpu

H = 32
D = 128
M = 512
SK = 4096
W = 1024
C = 512
HD = H * D
F32 = jnp.float32
BF16 = jnp.bfloat16
NT = (((1,), (1,)), ((), ()))

WO_GROUPS = (
    ((112,) * 9, 1040),
    ((112,), 1296),
    ((), 384),
    ((), 128),
)
WO_VPU = (96, 32)
NSLOT = 3
UNITS = tuple(u for g, _ in WO_GROUPS for u in g)
N_MAIN = 12 + len(WO_GROUPS) + len(WO_VPU)
assert sum(UNITS) + sum(r for _, r in WO_GROUPS) + sum(WO_VPU) == HD
assert sum(WO_VPU) <= D and all((sum(g) + r) % 128 == 0 for g, r in WO_GROUPS)


def _body(ax_hbm, ak_hbm, av_hbm, awq_hbm, awo_hbm, bx_hbm, bc_hbm, bwq_hbm, bwuk_hbm,
          bwuv_hbm, bwo_hbm, out_ref,
          ax_v, bx_v, k_v, v_v, awq_v, awo_v, c_v, bwq_v, bwuk_v, bwuv_v, bwo_v,
          acc_v, ocol_v, sm, sems, bsems):
    scale = 0.08837890625

    def scaled(s):
        return (s.astype(BF16).astype(F32) * scale).astype(BF16).astype(F32)

    hh = H // 2

    main = {}

    def mk(name, src, dst):
        main[name] = pltpu.make_async_copy(src, dst, sems.at[len(main)])

    mk('bwq', bwq_hbm, bwq_v)
    mk('bx', bx_hbm, bx_v)
    mk('ax', ax_hbm, ax_v)
    mk('bwuk', bwuk_hbm, bwuk_v)
    mk('c', bc_hbm, c_v)
    mk('awq', awq_hbm, awq_v)
    for name, src, dst in (('k', ak_hbm, k_v), ('v', av_hbm, v_v)):
        for i in range(2):
            mk(name + str(i), src.at[0, pl.ds(i * hh, hh), pl.ds(SK - W, W), :],
               dst.at[pl.ds(i * hh, hh)])
    mk('bwuv', bwuv_hbm, bwuv_v)
    mk('bwo', bwo_hbm, bwo_v)

    nu = len(UNITS)
    h2s, s2v = [], []
    r0 = 0
    for g, (units, direct) in enumerate(WO_GROUPS):
        for r in units:
            i = len(h2s)
            slot = sm.at[i % NSLOT, pl.ds(0, r), :]
            h2s.append(pltpu.make_async_copy(awo_hbm.at[pl.ds(r0, r), :], slot, bsems.at[i]))
            s2v.append(pltpu.make_async_copy(slot, awo_v.at[pl.ds(r0, r), :], bsems.at[nu + i]))
            r0 += r
        mk('wo%d' % g, awo_hbm.at[pl.ds(r0, direct), :], awo_v.at[pl.ds(r0, direct), :])
        r0 += direct
    for i, r in enumerate(WO_VPU):
        mk('wov%d' % i, awo_hbm.at[pl.ds(r0, r), :], awo_v.at[pl.ds(r0, r), :])
        r0 += r
    assert len(main) == N_MAIN

    n_sync = [0]
    s2v_done = set()

    def wait_s2v(i):
        if i not in s2v_done:
            s2v[i].wait()
            s2v_done.add(i)

    def sync():
        i = n_sync[0]
        n_sync[0] = i + 1
        if 1 <= i <= nu:
            h2s[i - 1].wait()
            s2v[i - 1].start()
        if i < nu:
            if i >= NSLOT:
                wait_s2v(i - NSLOT)
            h2s[i].start()

    def arrive(name):
        main[name].wait()
        sync()

    for cp in main.values():
        cp.start()
    sync()

    et = (lax.broadcasted_iota(jnp.int32, (128, 128 * H), 1) // H ==
          lax.broadcasted_iota(jnp.int32, (128, 128 * H), 0)).astype(BF16)
    dmask = (lax.broadcasted_iota(jnp.int32, (H, 128 * H), 1) % H ==
             lax.broadcasted_iota(jnp.int32, (H, 128 * H), 0))
    row8 = lax.broadcasted_iota(jnp.int32, (8, D), 0)

    def expand(y):
        ys = jnp.concatenate([y[:, t * 128:(t + 1) * 128] for t in range(4)], axis=0)
        ye = jnp.dot(ys, et, preferred_element_type=F32)
        return [jnp.where(dmask, ye[t * H:(t + 1) * H, :], 0.0).astype(BF16) for t in range(4)]

    def head_matmul(blocks, w_ref):
        acc = jnp.zeros((H, D), F32)
        for t in range(4):
            acc = acc + jnp.dot(blocks[t], w_ref[pl.ds(t * 128 * H, 128 * H), :],
                                preferred_element_type=F32)
        return acc

    arrive('bwq')
    main['bx'].wait()
    qb = head_matmul(expand(jnp.broadcast_to(bx_v[0], (H, M))), bwq_v).astype(BF16)

    arrive('bwuk')
    rm = []
    for t in range(4):
        r = lax.dot_general(qb, bwuk_v[pl.ds(t * 128 * H, 128 * H), :], NT,
                            preferred_element_type=F32)
        rm.append(jnp.where(dmask, r, 0.0).astype(BF16))
    qa_s = lax.dot_general(jnp.concatenate(rm, axis=0), et, NT, preferred_element_type=F32)
    qabs = jnp.concatenate([qa_s[t * H:(t + 1) * H, :] for t in range(4)], axis=1).astype(BF16)

    arrive('c')
    sb = scaled(lax.dot_general(qabs, c_v[...], NT, preferred_element_type=F32))
    eb = jnp.exp(sb - jnp.max(sb, axis=1, keepdims=True))
    lb = jnp.sum(eb, axis=1, keepdims=True)
    cc = jnp.dot(eb.astype(BF16), c_v[...], preferred_element_type=F32) / lb
    xv = expand(cc.astype(BF16))

    arrive('awq')
    main['ax'].wait()
    qa = jnp.dot(jnp.broadcast_to(ax_v[0], (8, M)), awq_v[...], preferred_element_type=F32)
    hmask = ((lax.broadcasted_iota(jnp.int32, (8, HD), 1) // D) % 8 ==
             lax.broadcasted_iota(jnp.int32, (8, HD), 0))
    qm = jnp.where(hmask, qa, 0.0).astype(BF16)

    arrive('k0')
    arrive('k1')
    ps = []
    for g in range(H // 8):
        s = jnp.zeros((8, W), F32)
        for h in range(8 * g, 8 * g + 8):
            s = s + lax.dot_general(qm[:, h * D:(h + 1) * D], k_v[h], NT,
                                    preferred_element_type=F32)
        s = scaled(s)
        e = jnp.exp(s - jnp.max(s, axis=1, keepdims=True))
        ps.append((e.astype(BF16), 1.0 / jnp.sum(e, axis=1, keepdims=True)))

    arrive('v0')
    arrive('v1')
    oms = []
    for h in range(H):
        e, inv = ps[h // 8]
        o = jnp.dot(e, v_v[h], preferred_element_type=F32) * inv
        oms.append(jnp.where(row8 == h % 8, o, 0.0).astype(BF16))
    om = jnp.concatenate(oms, axis=1)
    olast = oms[H - 1].astype(F32)[7:8, :]
    ocol_v[...] = jnp.broadcast_to(olast, (D, D)).T

    arrive('bwuv')
    cx = head_matmul(xv, bwuv_v)
    cxm = jnp.concatenate(
        [jnp.where(row8 == h % 8, cx[(h // 8) * 8:(h // 8) * 8 + 8, :], 0.0) for h in range(H)],
        axis=1).astype(BF16)
    arrive('bwo')
    ob = jnp.sum(jnp.dot(cxm, bwo_v[...], preferred_element_type=F32), axis=0, keepdims=True)
    out_ref[0, :, M:] = ob.astype(out_ref.dtype)

    assert n_sync[0] > nu
    r0 = 0
    u0 = 0
    for g, (units, direct) in enumerate(WO_GROUPS):
        main['wo%d' % g].wait()
        for i in range(u0, u0 + len(units)):
            wait_s2v(i)
        u0 += len(units)
        r = sum(units) + direct
        part = jnp.dot(om[:, r0:r0 + r], awo_v[pl.ds(r0, r), :], preferred_element_type=F32)
        acc_v[...] = part if g == 0 else part + acc_v[...]
        r0 += r
    for i, r in enumerate(WO_VPU):
        main['wov%d' % i].wait()
        part = acc_v[...]
        for rr in range(r0, r0 + r, 8):
            oc = ocol_v[pl.ds(rr - (HD - D), 8), :]
            part = part + (awo_v[pl.ds(rr, 8), :].astype(F32) *
                           jnp.concatenate([oc] * (M // D), axis=1))
        if i + 1 < len(WO_VPU):
            acc_v[...] = part
        else:
            out_ref[0, :, :M] = jnp.sum(part, axis=0, keepdims=True).astype(out_ref.dtype)
        r0 += r


def _kernel(*refs):
    pl.run_scoped(lambda sems, bsems: _body(*refs, sems, bsems),
                  pltpu.SemaphoreType.DMA((N_MAIN,)),
                  pltpu.SemaphoreType.DMA((2 * len(UNITS),)))


@jax.jit
def pallas_concat_heads__sliding_block_cached__compressed_kv_cla__decode_kernel(
    A_x: jax.Array,
    A_k_cache: jax.Array,
    A_v_cache: jax.Array,
    A_wq: jax.Array,
    A_wo: jax.Array,
    B_x: jax.Array,
    B_c_kv: jax.Array,
    B_w_q: jax.Array,
    B_w_uk: jax.Array,
    B_w_uv: jax.Array,
    B_w_o: jax.Array,
):
    return pl.pallas_call(
        _kernel,
        out_shape=jax.ShapeDtypeStruct((1, 1, 2 * M), BF16),
        in_specs=[pl.BlockSpec(memory_space=pl.ANY)] * 11,
        out_specs=pl.BlockSpec(memory_space=pltpu.VMEM),
        scratch_shapes=[
            pltpu.VMEM((1, 1, M), BF16),
            pltpu.VMEM((1, 1, M), BF16),
            pltpu.VMEM((H, W, D), BF16),
            pltpu.VMEM((H, W, D), BF16),
            pltpu.VMEM((M, HD), BF16),
            pltpu.VMEM((HD, M), BF16),
            pltpu.VMEM((SK, C), BF16),
            pltpu.VMEM((M * H, D), BF16),
            pltpu.VMEM((C * H, D), BF16),
            pltpu.VMEM((C * H, D), BF16),
            pltpu.VMEM((HD, M), BF16),
            pltpu.VMEM((8, M), F32),
            pltpu.VMEM((D, D), F32),
            pltpu.SMEM((NSLOT, max(UNITS), M), BF16),
        ],
        compiler_params=pltpu.CompilerParams(vmem_limit_bytes=100 * 1024 * 1024),
    )(A_x, A_k_cache, A_v_cache, A_wq, A_wo, B_x,
      B_c_kv.reshape(SK, C), B_w_q.reshape(M * H, D), B_w_uk.reshape(C * H, D),
      B_w_uv.reshape(C * H, D), B_w_o.reshape(HD, M))
```

```python
import jax
import jax.numpy as jnp
from jax import lax
import jax.experimental.pallas as pl
import jax.experimental.pallas.tpu as pltpu

H = 32
D = 128
M = 512
SK = 4096
W = 1024
C = 512
HD = H * D
F32 = jnp.float32
BF16 = jnp.bfloat16
NT = (((1,), (1,)), ((), ()))

G = 8
NSEG = 16
KV_SEGS = (128, 256, 128)

WO_GROUPS = (
    ((64,) + (128,) * 8, 960),
    ((128,), 1152),
    ((112,), 400),
    ((), 128),
)
WO_VPU = (96, 32)
NSLOT = 3
UNITS = tuple(u for g, _ in WO_GROUPS for u in g)
N_SEMS = 12 + len(WO_GROUPS) + len(WO_VPU) + 2 * len(UNITS)
assert sum(UNITS) + sum(r for _, r in WO_GROUPS) + sum(WO_VPU) == HD
assert sum(WO_VPU) <= D and all((sum(g) + r) % 128 == 0 for g, r in WO_GROUPS)


def _body(ax_hbm, ak_hbm, av_hbm, awq_hbm, awo_hbm, bx_hbm, bc_hbm, bwq_hbm, bwuk_hbm,
          bwuv_hbm, bwo_hbm, out_ref,
          ax_v, bx_v, k_v, v_v, awq_v, awo_v, c_v, bwq_v, bwuk_v, bwuv_v, bwo_v,
          acc_v, ocol_v, sm, sems):
    scale = 0.08837890625

    def scaled(s):
        return (s.astype(BF16).astype(F32) * scale).astype(BF16).astype(F32)

    n_sem = [0]

    def new_sem():
        n_sem[0] += 1
        return sems.at[n_sem[0] - 1]

    def copy(src, dst):
        return pltpu.make_async_copy(src, dst, new_sem())

    groups = []

    def add_group(src, dst, rows, ncol=1):
        sem = new_sem()
        cw = dst.shape[2] // ncol
        cps = []
        r0 = 0
        for r in rows:
            for c in range(ncol):
                idx = (slice(None), pl.ds(r0, r), pl.ds(c * cw, cw))
                cps.append(pltpu.make_async_copy(src.at[idx], dst.at[idx], sem))
            r0 += r
        assert r0 == dst.shape[1]
        groups.append((cps, pltpu.make_async_copy(dst, dst, sem)))

    def add_weight(src, dst):
        add_group(src, dst, (dst.shape[1] // NSEG,) * NSEG)

    add_weight(bwq_hbm, bwq_v)
    add_weight(bwuk_hbm, bwuk_v)
    add_weight(bc_hbm, c_v)
    add_group(awq_hbm, awq_v, (8,) * (M // G // 8), ncol=2)
    for src, dst in ((ak_hbm, k_v), (av_hbm, v_v)):
        for i in range(2):
            add_group(src.at[0, :, pl.ds(SK - W + i * (W // 2), W // 2), :],
                      dst.at[:, pl.ds(i * (W // 2), W // 2), :], KV_SEGS)
    add_weight(bwuv_hbm, bwuv_v)
    add_weight(bwo_hbm, bwo_v)
    bx_cp = copy(bx_hbm, bx_v)
    ax_cp = copy(ax_hbm, ax_v)

    nu = len(UNITS)
    h2s, s2v, wo_cps = [], [], []
    r0 = 0
    for units, direct in WO_GROUPS + tuple(((), r) for r in WO_VPU):
        for r in units:
            slot = sm.at[len(h2s) % NSLOT, pl.ds(0, r), :]
            h2s.append(copy(awo_hbm.at[pl.ds(r0, r), :], slot))
            s2v.append(copy(slot, awo_v.at[pl.ds(r0, r), :]))
            r0 += r
        wo_cps.append(copy(awo_hbm.at[pl.ds(r0, direct), :], awo_v.at[pl.ds(r0, direct), :]))
        r0 += direct
    assert n_sem[0] == N_SEMS
    batches = [cps for cps, _ in groups] + [wo_cps]

    s2v_done = set()

    def wait_s2v(i):
        if i not in s2v_done:
            s2v[i].wait()
            s2v_done.add(i)

    def forward(i):
        h2s[i].wait()
        s2v[i].start()

    def fetch(i):
        if i >= NSLOT:
            wait_s2v(i - NSLOT)
        h2s[i].start()

    n_arrived = [0]

    def arrive():
        n = n_arrived[0]
        n_arrived[0] = n + 1
        groups[n][1].wait()
        if n + 2 < nu:
            fetch(n + 2)
        if n + 1 < nu:
            forward(n + 1)
        if n + 2 < len(batches):
            for cp in batches[n + 2]:
                cp.start()

    batches[0][0].start()
    fetch(0)
    fetch(1)
    for cp in batches[0][1:] + [bx_cp, ax_cp]:
        cp.start()
    forward(0)
    for cp in batches[1]:
        cp.start()

    et = (lax.broadcasted_iota(jnp.int32, (128, 128 * H), 1) // H ==
          lax.broadcasted_iota(jnp.int32, (128, 128 * H), 0)).astype(BF16)
    dmask = (lax.broadcasted_iota(jnp.int32, (H, 128 * H), 1) % H ==
             lax.broadcasted_iota(jnp.int32, (H, 128 * H), 0))
    row8 = lax.broadcasted_iota(jnp.int32, (8, D), 0)

    def rows2d(ref, t=None):
        x = ref[...] if t is None else ref[pl.ds(t * (G // 4), G // 4)]
        return x.reshape(x.shape[0] * x.shape[1], x.shape[2])

    def expand(y):
        ys = jnp.concatenate([y[:, t * 128:(t + 1) * 128] for t in range(4)], axis=0)
        ye = jnp.dot(ys, et, preferred_element_type=F32)
        return [jnp.where(dmask, ye[t * H:(t + 1) * H, :], 0.0).astype(BF16) for t in range(4)]

    def head_matmul(blocks, w_ref):
        acc = jnp.zeros((H, D), F32)
        for t in range(4):
            acc = acc + jnp.dot(blocks[t], rows2d(w_ref, t), preferred_element_type=F32)
        return acc

    arrive()
    bx_cp.wait()
    qb = head_matmul(expand(jnp.broadcast_to(bx_v[0], (H, M))), bwq_v).astype(BF16)

    arrive()
    rm = []
    for t in range(4):
        r = lax.dot_general(qb, rows2d(bwuk_v, t), NT, preferred_element_type=F32)
        rm.append(jnp.where(dmask, r, 0.0).astype(BF16))
    qa_s = lax.dot_general(jnp.concatenate(rm, axis=0), et, NT, preferred_element_type=F32)
    qabs = jnp.concatenate([qa_s[t * H:(t + 1) * H, :] for t in range(4)], axis=1).astype(BF16)

    arrive()
    sb = scaled(lax.dot_general(qabs, rows2d(c_v), NT, preferred_element_type=F32))
    eb = jnp.exp(sb - jnp.max(sb, axis=1, keepdims=True))
    lb = jnp.sum(eb, axis=1, keepdims=True)
    cc = jnp.dot(eb.astype(BF16), rows2d(c_v), preferred_element_type=F32) / lb
    xv = expand(cc.astype(BF16))

    arrive()
    ax_cp.wait()
    qa = jnp.dot(jnp.broadcast_to(ax_v[0], (8, M)), rows2d(awq_v), preferred_element_type=F32)
    hmask = ((lax.broadcasted_iota(jnp.int32, (8, HD), 1) // D) % 8 ==
             lax.broadcasted_iota(jnp.int32, (8, HD), 0))
    qm = jnp.where(hmask, qa, 0.0).astype(BF16)

    arrive()
    arrive()
    ps = []
    for g in range(H // 8):
        s = jnp.zeros((8, W), F32)
        for h in range(8 * g, 8 * g + 8):
            s = s + lax.dot_general(qm[:, h * D:(h + 1) * D], k_v[h], NT,
                                    preferred_element_type=F32)
        s = scaled(s)
        e = jnp.exp(s - jnp.max(s, axis=1, keepdims=True))
        ps.append((e.astype(BF16), 1.0 / jnp.sum(e, axis=1, keepdims=True)))

    arrive()
    arrive()
    oms = []
    for h in range(H):
        e, inv = ps[h // 8]
        o = jnp.dot(e, v_v[h], preferred_element_type=F32) * inv
        oms.append(jnp.where(row8 == h % 8, o, 0.0).astype(BF16))
    om = jnp.concatenate(oms, axis=1)
    olast = oms[H - 1].astype(F32)[7:8, :]
    ocol_v[...] = jnp.broadcast_to(olast, (D, D)).T

    arrive()
    cx = head_matmul(xv, bwuv_v)
    cxm = jnp.concatenate(
        [jnp.where(row8 == h % 8, cx[(h // 8) * 8:(h // 8) * 8 + 8, :], 0.0) for h in range(H)],
        axis=1).astype(BF16)
    arrive()
    ob = jnp.sum(jnp.dot(cxm, rows2d(bwo_v), preferred_element_type=F32), axis=0, keepdims=True)
    out_ref[0, :, M:] = ob.astype(out_ref.dtype)

    assert n_arrived[0] == len(groups) >= nu - 1
    r0 = 0
    u0 = 0
    for g, (units, direct) in enumerate(WO_GROUPS):
        wo_cps[g].wait()
        for i in range(u0, u0 + len(units)):
            wait_s2v(i)
        u0 += len(units)
        r = sum(units) + direct
        part = jnp.dot(om[:, r0:r0 + r], awo_v[pl.ds(r0, r), :], preferred_element_type=F32)
        acc_v[...] = part if g == 0 else part + acc_v[...]
        r0 += r
    for i, r in enumerate(WO_VPU):
        wo_cps[len(WO_GROUPS) + i].wait()
        part = acc_v[...]
        for rr in range(r0, r0 + r, 8):
            oc = ocol_v[pl.ds(rr - (HD - D), 8), :]
            part = part + (awo_v[pl.ds(rr, 8), :].astype(F32) *
                           jnp.concatenate([oc] * (M // D), axis=1))
        if i + 1 < len(WO_VPU):
            acc_v[...] = part
        else:
            out_ref[0, :, :M] = jnp.sum(part, axis=0, keepdims=True).astype(out_ref.dtype)
        r0 += r


def _kernel(*refs):
    pl.run_scoped(lambda sems: _body(*refs, sems), pltpu.SemaphoreType.DMA((N_SEMS,)))


@jax.jit
def pallas_concat_heads__sliding_block_cached__compressed_kv_cla__decode_kernel(
    A_x: jax.Array,
    A_k_cache: jax.Array,
    A_v_cache: jax.Array,
    A_wq: jax.Array,
    A_wo: jax.Array,
    B_x: jax.Array,
    B_c_kv: jax.Array,
    B_w_q: jax.Array,
    B_w_uk: jax.Array,
    B_w_uv: jax.Array,
    B_w_o: jax.Array,
):
    views = dict(awq=(G, M // G, HD), c=(G, SK // G, C), w=(G, M * H // G, D), bwo=(G, HD // G, M))
    return pl.pallas_call(
        _kernel,
        out_shape=jax.ShapeDtypeStruct((1, 1, 2 * M), BF16),
        in_specs=[pl.BlockSpec(memory_space=pl.ANY)] * 11,
        out_specs=pl.BlockSpec(memory_space=pltpu.VMEM),
        scratch_shapes=[
            pltpu.VMEM((1, 1, M), BF16),
            pltpu.VMEM((1, 1, M), BF16),
            pltpu.VMEM((H, W, D), BF16),
            pltpu.VMEM((H, W, D), BF16),
            pltpu.VMEM(views['awq'], BF16),
            pltpu.VMEM((HD, M), BF16),
            pltpu.VMEM(views['c'], BF16),
            pltpu.VMEM(views['w'], BF16),
            pltpu.VMEM(views['w'], BF16),
            pltpu.VMEM(views['w'], BF16),
            pltpu.VMEM(views['bwo'], BF16),
            pltpu.VMEM((8, M), F32),
            pltpu.VMEM((D, D), F32),
            pltpu.SMEM((NSLOT, max(UNITS), M), BF16),
        ],
        compiler_params=pltpu.CompilerParams(vmem_limit_bytes=100 * 1024 * 1024),
    )(A_x, A_k_cache, A_v_cache, A_wq.reshape(views['awq']), A_wo, B_x,
      B_c_kv.reshape(views['c']), B_w_q.reshape(views['w']), B_w_uk.reshape(views['w']),
      B_w_uv.reshape(views['w']), B_w_o.reshape(views['bwo']))
```

```python
import jax
import jax.numpy as jnp
from jax import lax
import jax.experimental.pallas as pl
import jax.experimental.pallas.tpu as pltpu

H = 32
D = 128
M = 512
SK = 4096
W = 1024
C = 512
HD = H * D
F32 = jnp.float32
BF16 = jnp.bfloat16
NT = (((1,), (1,)), ((), ()))

G = 8
W_PIECES = (1,) + (2,) * 7 + (1,)
KV_PIECES = (128, 256, 256, 256, 128)

WO_GROUPS = (
    ((128,) * 9, 896),
    ((128,), 1152),
    ((80,), 432),
    ((), 128),
)
WO_VPU = (96, 32)
NSLOT = 3
UNITS = tuple(u for g, _ in WO_GROUPS for u in g)
N_SEMS = 12 + len(WO_GROUPS) + len(WO_VPU) + 2 * len(UNITS)
assert sum(UNITS) + sum(r for _, r in WO_GROUPS) + sum(WO_VPU) == HD
assert sum(WO_VPU) <= D and all((sum(g) + r) % 128 == 0 for g, r in WO_GROUPS)


def _body(ax_hbm, ak_hbm, av_hbm, awq_hbm, awo_hbm, bx_hbm, bc_hbm, bwq_hbm, bwuk_hbm,
          bwuv_hbm, bwo_hbm, out_ref,
          ax_v, bx_v, k_v, v_v, awq_v, awo_v, c_v, bwq_v, bwuk_v, bwuv_v, bwo_v,
          acc_v, ocol_v, sm, sems):
    scale = 0.08837890625

    def scaled(s):
        return (s.astype(BF16).astype(F32) * scale).astype(BF16).astype(F32)

    n_sem = [0]

    def new_sem():
        n_sem[0] += 1
        return sems.at[n_sem[0] - 1]

    def copy(src, dst):
        return pltpu.make_async_copy(src, dst, new_sem())

    groups = []

    def add_group(src, dst, rows, ncol=1):
        sem = new_sem()
        cw = dst.shape[2] // ncol
        cps = []
        r0 = 0
        for r in rows:
            for c in range(ncol):
                idx = (slice(None), pl.ds(r0, r), pl.ds(c * cw, cw))
                cps.append(pltpu.make_async_copy(src.at[idx], dst.at[idx], sem))
            r0 += r
        assert r0 == dst.shape[1]
        groups.append((cps, pltpu.make_async_copy(dst, dst, sem)))

    def add_weight(src, dst):
        add_group(src, dst, tuple(dst.shape[1] // 16 * p for p in W_PIECES))

    add_weight(bwq_hbm, bwq_v)
    add_weight(bwuk_hbm, bwuk_v)
    add_weight(bc_hbm, c_v)
    add_group(awq_hbm, awq_v, (8,) * (M // G // 8), ncol=2)
    for src, dst in ((ak_hbm, k_v), (av_hbm, v_v)):
        for i in range(2):
            add_group(src.at[0, pl.ds(i * (H // 2), H // 2), pl.ds(SK - W, W), :],
                      dst.at[pl.ds(i * (H // 2), H // 2)], KV_PIECES)
    add_weight(bwuv_hbm, bwuv_v)
    add_weight(bwo_hbm, bwo_v)
    bx_cp = copy(bx_hbm, bx_v)
    ax_cp = copy(ax_hbm, ax_v)

    nu = len(UNITS)
    h2s, s2v, wo_cps = [], [], []
    r0 = 0
    for units, direct in WO_GROUPS + tuple(((), r) for r in WO_VPU):
        for r in units:
            slot = sm.at[len(h2s) % NSLOT, pl.ds(0, r), :]
            h2s.append(copy(awo_hbm.at[pl.ds(r0, r), :], slot))
            s2v.append(copy(slot, awo_v.at[pl.ds(r0, r), :]))
            r0 += r
        wo_cps.append(copy(awo_hbm.at[pl.ds(r0, direct), :], awo_v.at[pl.ds(r0, direct), :]))
        r0 += direct
    assert n_sem[0] == N_SEMS
    batches = [cps for cps, _ in groups] + [wo_cps]

    s2v_done = set()

    def wait_s2v(i):
        if i not in s2v_done:
            s2v[i].wait()
            s2v_done.add(i)

    def forward(i):
        h2s[i].wait()
        s2v[i].start()

    def fetch(i):
        if i >= NSLOT:
            wait_s2v(i - NSLOT)
        h2s[i].start()

    n_arrived = [0]

    def arrive():
        n = n_arrived[0]
        n_arrived[0] = n + 1
        groups[n][1].wait()
        if n + 2 < nu:
            fetch(n + 2)
        if n + 1 < nu:
            forward(n + 1)
        if n + 2 < len(batches):
            for cp in batches[n + 2]:
                cp.start()

    batches[0][0].start()
    fetch(0)
    fetch(1)
    for cp in batches[0][1:] + [bx_cp, ax_cp] + batches[1]:
        cp.start()
    forward(0)

    et = (lax.broadcasted_iota(jnp.int32, (128, 128 * H), 1) // H ==
          lax.broadcasted_iota(jnp.int32, (128, 128 * H), 0)).astype(BF16)
    dmask = (lax.broadcasted_iota(jnp.int32, (H, 128 * H), 1) % H ==
             lax.broadcasted_iota(jnp.int32, (H, 128 * H), 0))
    row8 = lax.broadcasted_iota(jnp.int32, (8, D), 0)

    def rows2d(ref, t=None):
        x = ref[...] if t is None else ref[pl.ds(t * (G // 4), G // 4)]
        return x.reshape(x.shape[0] * x.shape[1], x.shape[2])

    def expand(y):
        ys = jnp.concatenate([y[:, t * 128:(t + 1) * 128] for t in range(4)], axis=0)
        ye = jnp.dot(ys, et, preferred_element_type=F32)
        return [jnp.where(dmask, ye[t * H:(t + 1) * H, :], 0.0).astype(BF16) for t in range(4)]

    def head_matmul(blocks, w_ref):
        acc = jnp.zeros((H, D), F32)
        for t in range(4):
            acc = acc + jnp.dot(blocks[t], rows2d(w_ref, t), preferred_element_type=F32)
        return acc

    arrive()
    bx_cp.wait()
    qb = head_matmul(expand(jnp.broadcast_to(bx_v[0], (H, M))), bwq_v).astype(BF16)

    arrive()
    rm = []
    for t in range(4):
        r = lax.dot_general(qb, rows2d(bwuk_v, t), NT, preferred_element_type=F32)
        rm.append(jnp.where(dmask, r, 0.0).astype(BF16))
    qa_s = lax.dot_general(jnp.concatenate(rm, axis=0), et, NT, preferred_element_type=F32)
    qabs = jnp.concatenate([qa_s[t * H:(t + 1) * H, :] for t in range(4)], axis=1).astype(BF16)

    arrive()
    sb = scaled(lax.dot_general(qabs, rows2d(c_v), NT, preferred_element_type=F32))
    eb = jnp.exp(sb - jnp.max(sb, axis=1, keepdims=True))
    lb = jnp.sum(eb, axis=1, keepdims=True)
    cc = jnp.dot(eb.astype(BF16), rows2d(c_v), preferred_element_type=F32) / lb
    xv = expand(cc.astype(BF16))

    arrive()
    ax_cp.wait()
    qa = jnp.dot(jnp.broadcast_to(ax_v[0], (8, M)), rows2d(awq_v), preferred_element_type=F32)
    hmask = ((lax.broadcasted_iota(jnp.int32, (8, HD), 1) // D) % 8 ==
             lax.broadcasted_iota(jnp.int32, (8, HD), 0))
    qm = jnp.where(hmask, qa, 0.0).astype(BF16)

    arrive()
    arrive()
    ps = []
    for g in range(H // 8):
        s = jnp.zeros((8, W), F32)
        for h in range(8 * g, 8 * g + 8):
            s = s + lax.dot_general(qm[:, h * D:(h + 1) * D], k_v[h], NT,
                                    preferred_element_type=F32)
        s = scaled(s)
        e = jnp.exp(s - jnp.max(s, axis=1, keepdims=True))
        ps.append((e.astype(BF16), 1.0 / jnp.sum(e, axis=1, keepdims=True)))

    arrive()
    arrive()
    oms = []
    for h in range(H):
        e, inv = ps[h // 8]
        o = jnp.dot(e, v_v[h], preferred_element_type=F32) * inv
        oms.append(jnp.where(row8 == h % 8, o, 0.0).astype(BF16))
    om = jnp.concatenate(oms, axis=1)
    olast = oms[H - 1].astype(F32)[7:8, :]
    ocol_v[...] = jnp.broadcast_to(olast, (D, D)).T

    arrive()
    cx = head_matmul(xv, bwuv_v)
    cxm = jnp.concatenate(
        [jnp.where(row8 == h % 8, cx[(h // 8) * 8:(h // 8) * 8 + 8, :], 0.0) for h in range(H)],
        axis=1).astype(BF16)
    arrive()
    ob = jnp.sum(jnp.dot(cxm, rows2d(bwo_v), preferred_element_type=F32), axis=0, keepdims=True)
    out_ref[0, :, M:] = ob.astype(out_ref.dtype)

    assert n_arrived[0] == len(groups) >= nu - 1
    r0 = 0
    u0 = 0
    for g, (units, direct) in enumerate(WO_GROUPS):
        wo_cps[g].wait()
        for i in range(u0, u0 + len(units)):
            wait_s2v(i)
        u0 += len(units)
        r = sum(units) + direct
        part = jnp.dot(om[:, r0:r0 + r], awo_v[pl.ds(r0, r), :], preferred_element_type=F32)
        acc_v[...] = part if g == 0 else part + acc_v[...]
        r0 += r
    for i, r in enumerate(WO_VPU):
        wo_cps[len(WO_GROUPS) + i].wait()
        part = acc_v[...]
        for rr in range(r0, r0 + r, 8):
            oc = ocol_v[pl.ds(rr - (HD - D), 8), :]
            part = part + (awo_v[pl.ds(rr, 8), :].astype(F32) *
                           jnp.concatenate([oc] * (M // D), axis=1))
        if i + 1 < len(WO_VPU):
            acc_v[...] = part
        else:
            out_ref[0, :, :M] = jnp.sum(part, axis=0, keepdims=True).astype(out_ref.dtype)
        r0 += r


def _kernel(*refs):
    pl.run_scoped(lambda sems: _body(*refs, sems), pltpu.SemaphoreType.DMA((N_SEMS,)))


@jax.jit
def pallas_concat_heads__sliding_block_cached__compressed_kv_cla__decode_kernel(
    A_x: jax.Array,
    A_k_cache: jax.Array,
    A_v_cache: jax.Array,
    A_wq: jax.Array,
    A_wo: jax.Array,
    B_x: jax.Array,
    B_c_kv: jax.Array,
    B_w_q: jax.Array,
    B_w_uk: jax.Array,
    B_w_uv: jax.Array,
    B_w_o: jax.Array,
):
    views = dict(awq=(G, M // G, HD), c=(G, SK // G, C), w=(G, M * H // G, D), bwo=(G, HD // G, M))
    return pl.pallas_call(
        _kernel,
        out_shape=jax.ShapeDtypeStruct((1, 1, 2 * M), BF16),
        in_specs=[pl.BlockSpec(memory_space=pl.ANY)] * 11,
        out_specs=pl.BlockSpec(memory_space=pltpu.VMEM),
        scratch_shapes=[
            pltpu.VMEM((1, 1, M), BF16),
            pltpu.VMEM((1, 1, M), BF16),
            pltpu.VMEM((H, W, D), BF16),
            pltpu.VMEM((H, W, D), BF16),
            pltpu.VMEM(views['awq'], BF16),
            pltpu.VMEM((HD, M), BF16),
            pltpu.VMEM(views['c'], BF16),
            pltpu.VMEM(views['w'], BF16),
            pltpu.VMEM(views['w'], BF16),
            pltpu.VMEM(views['w'], BF16),
            pltpu.VMEM(views['bwo'], BF16),
            pltpu.VMEM((8, M), F32),
            pltpu.VMEM((D, D), F32),
            pltpu.SMEM((NSLOT, max(UNITS), M), BF16),
        ],
        compiler_params=pltpu.CompilerParams(vmem_limit_bytes=100 * 1024 * 1024),
    )(A_x, A_k_cache, A_v_cache, A_wq.reshape(views['awq']), A_wo, B_x,
      B_c_kv.reshape(views['c']), B_w_q.reshape(views['w']), B_w_uk.reshape(views['w']),
      B_w_uv.reshape(views['w']), B_w_o.reshape(views['bwo']))
```
